```python
import os as _os
_os.environ.setdefault("JAX_PLATFORMS", "cpu")
import jax
import jax.numpy as jnp

def _softmax(x, axis=-1):
    return jax.nn.softmax(x, axis=axis)
def _gelu(x):
    return jax.nn.gelu(x, approximate=True)
def _silu(x):
    return jax.nn.silu(x)
def _sigmoid(x):
    return jax.nn.sigmoid(x)
def _layernorm(x, axis=-1, eps=1e-5):
    m = jnp.mean(x, axis=axis, keepdims=True)
    v = jnp.var(x, axis=axis, keepdims=True)
    return (x - m) / jnp.sqrt(v + eps)
def _scatter_add(tgt, idx, src, axis=0):
    return tgt.at[idx].add(src)
def _segment_sum(src, seg, n):
    return jax.ops.segment_sum(src, seg, n)
class _Rng:
    def __init__(self, key):
        self._k = key
    def _next(self):
        self._k, sub = jax.random.split(self._k)
        return sub
    def normal(self, shape):
        return jax.random.normal(self._next(), shape, dtype=jnp.bfloat16)
    def randint(self, lo, hi, shape):
        return jax.random.randint(self._next(), shape, lo, hi, dtype=jnp.int32)
    def uniform(self, shape, lo=0.0, hi=1.0):
        return jax.random.uniform(self._next(), shape, jnp.bfloat16, lo, hi)
    def permutation(self, n):
        return jax.random.permutation(self._next(), n)


kernel_name = 'gated_mix__ssm_conv_s5__glu_gated_geglu__prompt'

def setup_inputs():
    _rng = _Rng(jax.random.key(int.from_bytes(__import__("os").urandom(4), "little")))
    _w = (lambda a: (lambda t: t.astype(jnp.bfloat16) if jnp.issubdtype(t.dtype, jnp.floating) else t)(jnp.asarray(a)))
    def _A_setup():
        B, S, D = 1, 2048, 1024
        P = D
        Lambda_re = -0.5 * jnp.exp((lambda *s: _rng.normal(s) * 0.4)(P))
        Lambda_im = (lambda *s: _rng.normal(s) * 0.4)(P) * 1.0
        B_re = (lambda *s: _rng.normal(s) * 0.4)(P, D) * (D ** -0.5)
        B_im = (lambda *s: _rng.normal(s) * 0.4)(P, D) * (D ** -0.5)
        C_re = (lambda *s: _rng.normal(s) * 0.4)(D, P) * (P ** -0.5)
        C_im = (lambda *s: _rng.normal(s) * 0.4)(D, P) * (P ** -0.5)
        log_dt = (lambda *s: _rng.normal(s) * 0.4)(P) * 0.3 - 2.0
        Dskip = (lambda *s: _rng.normal(s) * 0.4)(D)
        return {
            "x": _w((lambda *s: _rng.normal(s) * 0.05)(B, S, D)),
            "Lambda_re": _w(Lambda_re),
            "Lambda_im": _w(Lambda_im),
            "B_re": _w(B_re),
            "B_im": _w(B_im),
            "C_re": _w(C_re),
            "C_im": _w(C_im),
            "log_dt": _w(log_dt),
            "Dskip": _w(Dskip),
        }
    _A_in = _A_setup()

    def _B_setup():
        B, S, Dm, Df = 1, 2048, 1024, 3584
        return {
            "x": _w((lambda *s: _rng.normal(s) * 0.05)(B, S, Dm)),
            "w_gate": _w((lambda *s: _rng.normal(s) * 1.6)(Dm, Df) * (Dm ** -0.5)),
            "w_up": _w((lambda *s: _rng.normal(s) * 1.6)(Dm, Df) * (Dm ** -0.5)),
            "w_down": _w((lambda *s: _rng.normal(s) * 1.6)(Df, Dm) * (Df ** -0.5)),
        }
    _B_in = _B_setup()

    return {
        "A_x": _A_in["x"],
        "A_Lambda_re": _A_in["Lambda_re"],
        "A_Lambda_im": _A_in["Lambda_im"],
        "A_B_re": _A_in["B_re"],
        "A_B_im": _A_in["B_im"],
        "A_C_re": _A_in["C_re"],
        "A_C_im": _A_in["C_im"],
        "A_log_dt": _A_in["log_dt"],
        "A_Dskip": _A_in["Dskip"],
        "B_x": _B_in["x"],
        "B_w_gate": _B_in["w_gate"],
        "B_w_up": _B_in["w_up"],
        "B_w_down": _B_in["w_down"],
        "gate_w": _w((lambda *s: _rng.normal(s) * 0.05)(1024) * 16.0),
    }

def reference(A_x, A_Lambda_re, A_Lambda_im, A_B_re, A_B_im, A_C_re, A_C_im, A_log_dt, A_Dskip, B_x, B_w_gate, B_w_up, B_w_down, gate_w):
    def _A_ref(x, Lambda_re, Lambda_im, B_re, B_im, C_re, C_im, log_dt, Dskip):
        Bsz, L, H = x.shape
        Lam = Lambda_re + 1j * Lambda_im
        Bmat = B_re + 1j * B_im
        Cmat = C_re + 1j * C_im
        dt = jnp.exp(log_dt)
        Lam_bar = jnp.exp(dt * Lam)
        B_bar = ((Lam_bar - 1.0) / Lam)[:, None] * Bmat
        Bu = jnp.einsum("bld,pd->blp", x + 0j, B_bar)
        h = jnp.zeros_like(Bu[:, 0, :])
        hs = []
        for t in range(L):
            h = Lam_bar[None, :] * h + Bu[:, t, :]
            hs.append(h)
        hseq = jnp.stack(hs, 1)
        y = 2.0 * jnp.einsum("blp,dp->bld", hseq, Cmat).real + x * Dskip[None, None, :]
        return y

    def _B_ref(x, w_gate, w_up, w_down):
        g = jnp.einsum("bsd,df->bsf", x, w_gate)
        u = jnp.einsum("bsd,df->bsf", x, w_up)
        h = _gelu(g) * u
        return jnp.einsum("bsf,fd->bsd", h, w_down)

    x = A_x
    g = _sigmoid((x * gate_w).sum(-1, keepdims=True))
    a = _A_ref(x, A_Lambda_re, A_Lambda_im, A_B_re, A_B_im, A_C_re, A_C_im, A_log_dt, A_Dskip)
    b = _B_ref(x, B_w_gate, B_w_up, B_w_down)
    return g * a + (1 - g) * b
```

```python
import jax
import jax.numpy as jnp
from jax import lax
from jax.experimental import pallas as pl
from jax.experimental.pallas import tpu as pltpu

_L, _D, _P, _F = 2048, 1024, 1024, 3584
_R = 256
_NBLK = _L // _R
_FC = 512
_NO = 256
_S = _L + 4
_GR = _R // 8
_SX0, _SX1, _SXR, _SB, _SV, _SW, _NSEM = 0, 1, 2, 3, 19, 24, 29

_f32, _bf16, _u32 = jnp.float32, jnp.bfloat16, jnp.uint32


def _dot(a, b):
    return jnp.dot(a, b, preferred_element_type=_f32)


def _dot_nt(a, b):
    return lax.dot_general(a, b, (((1,), (1,)), ((), ())), preferred_element_type=_f32)


def _gelu(x):
    c = 0.7978845608028654
    return 0.5 * x * (1.0 + jnp.tanh(c * (x + 0.044715 * (x * x * x))))


def _align(v, m):
    return v if isinstance(v, int) else pl.multiple_of(v, m)


def _tile(v, n):
    return jnp.concatenate([v] * n, axis=0)


def _kernel(x_hbm, lre_hbm, lim_hbm, ldt_hbm, dsk_hbm, gw_hbm,
            bre_hbm, bim_hbm, cre_hbm, cim_hbm, wg_hbm, wu_hbm, wd_hbm, o_hbm,
            xs, bre_s, bim_s, cre_s, cim_s, wg_s, wu_s, wd_s, vec_s,
            par, dk, cf, gs, bur, bui, hre, him, hg, ost, sem, sem_o):
    R, S = _R, _S

    def rows_copy(r0, nr, k):
        return pltpu.make_async_copy(x_hbm.at[pl.ds(r0, nr), :], xs.at[pl.ds(r0, nr), :], sem.at[k])

    def x_copies():
        return rows_copy(0, R, _SX0), rows_copy(R, R, _SX1), rows_copy(2 * R, _L - 2 * R, _SXR)

    def b_copy(l, k):
        src, dst = ((bre_hbm, bre_s), (bim_hbm, bim_s))[k]
        rows = pl.ds(_align(l * 128, 128), 128)
        return pltpu.make_async_copy(src.at[rows, :], dst.at[rows, :], sem.at[_SB + 2 * l + k])

    def b_copies(l):
        return [b_copy(l, 0), b_copy(l, 1)]

    def vec_copies():
        return [pltpu.make_async_copy(v, vec_s.at[k], sem.at[_SV + k])
                for k, v in enumerate((lre_hbm, lim_hbm, ldt_hbm, dsk_hbm, gw_hbm))]

    def w_copies():
        return [pltpu.make_async_copy(src, dst, sem.at[_SW + k]) for k, (src, dst) in enumerate(
            ((wg_hbm, wg_s), (wu_hbm, wu_s), (cre_hbm, cre_s), (cim_hbm, cim_s), (wd_hbm, wd_s)))]

    def start(cs):
        for c in cs:
            c.start()

    def wait(cs):
        for c in cs:
            c.wait()

    x0c, x1c, xrc = x_copies()
    start([x0c] + b_copies(0) + vec_copies() + [x1c])
    for l in range(1, 8):
        start(b_copies(l))
    start([xrc] + w_copies())

    def params():
        lre = vec_s[0].astype(_f32)
        lim = vec_s[1].astype(_f32)
        dt = jnp.exp(vec_s[2].astype(_f32)).astype(_bf16).astype(_f32)
        mag = jnp.exp(dt * lre)
        ang = dt * lim
        ar = mag * jnp.cos(ang)
        ai = mag * jnp.sin(ang)
        nr = ar - 1.0
        den = 2.0 / (lre * lre + lim * lim)
        cr = (nr * lre + ai * lim) * den
        ci = (ai * lre - nr * lim) * den
        par[0] = ar
        par[1] = ai
        dsk = vec_s[3].astype(_f32)
        gw = vec_s[4].astype(_f32)
        for l in range(8):
            sl = slice(l * 128, (l + 1) * 128)
            dk[0, :, sl] = jnp.broadcast_to(dsk[l:l + 1, :], (8, 128))
            dk[1, :, sl] = jnp.broadcast_to(gw[l:l + 1, :], (8, 128))
            cf[0, l] = jnp.broadcast_to(cr[l:l + 1, :], (8, 128))
            cf[1, l] = jnp.broadcast_to(ci[l:l + 1, :], (8, 128))

    def gate_rows(r0, nr):
        xf = xs[pl.ds(r0, nr), :].astype(_f32)
        s = jnp.sum(xf * _tile(dk[1], nr // 8), axis=-1, keepdims=True)
        g = jnp.broadcast_to(jax.nn.sigmoid(s), (nr, 128))
        gs[pl.ds(r0, nr), :] = g
        return g

    def bu_dot(r0, l):
        x = xs[pl.ds(r0, R), :]
        rows = pl.ds(_align(l * 128, 128), 128)
        return _dot_nt(x, bre_s[rows, :]), _dot_nt(x, bim_s[rows, :])

    def bu_fin(r0, l0, k, b_r, b_i):
        l = l0 + k
        c_r = cf[0, l]
        c_i = cf[1, l]
        g = gate_rows(_align(r0 + l * _GR, _GR), _GR)
        w = lax.bitcast_convert_type(g, _u32)
        m = w[0:8]
        for j in range(1, _GR // 8):
            m = m | w[8 * j:8 * j + 8]
        c_r = jnp.where((m | 1) != 0, c_r, 0.0)
        c_r = _tile(c_r, R // 8)
        c_i = _tile(c_i, R // 8)
        base = _align(l0 * S + r0 + (k * S // 8) * 8, 8) + (k * S) % 8
        bur[pl.ds(base, R), :] = c_r * b_r - c_i * b_i
        bui[pl.ds(base, R), :] = -(c_r * b_i + c_i * b_r)

    def bu(r0, l0, k):
        bu_fin(r0, l0, k, *bu_dot(r0, l0 + k))

    x0c, x1c, xrc = x_copies()
    wait([x0c] + b_copies(0))
    first = bu_dot(0, 0)
    wait([x1c] + vec_copies())
    params()
    bu_fin(0, 0, 0, *first)
    bu(R, 0, 0)
    wait(b_copies(1))
    bu(0, 0, 1)
    bu(R, 0, 1)

    def p0(j, c):
        l0 = 2 * j
        wait(b_copies(l0) + b_copies(l0 + 1))
        for k in range(2):
            bu(0, l0, k)
            bu(R, l0, k)
        return c

    lax.fori_loop(1, 4, p0, 0)
    wait([xrc])

    def p1(i, c):
        r0 = pl.multiple_of(i * R, R)
        for l in range(8):
            bu(r0, 0, l)
        return c

    lax.fori_loop(2, _NBLK, p1, 0)

    def scan(r0, hr, hi):
        ar, ai = par[0], par[1]
        for t in range(R):
            b_r = bur[pl.ds(r0 + t, 8, stride=S), :]
            b_i = bui[pl.ds(r0 + t, 8, stride=S), :]
            hr, hi = ar * hr + ai * hi + b_r, ar * hi - ai * hr + b_i
            hre[pl.ds(r0 + t, 8, stride=S), :] = hr
            him[pl.ds(r0 + t, 8, stride=S), :] = hi
        return hr, hi

    def hidden(r0):
        x = xs[pl.ds(r0, R), :]
        for f0 in range(0, _F, _FC):
            g = _dot(x, wg_s[:, f0:f0 + _FC])
            u = _dot(x, wu_s[:, f0:f0 + _FC])
            hg[pl.ds(r0, R), f0:f0 + _FC] = (_gelu(g) * u).astype(_bf16)

    def loop_a(i, carry):
        r0 = pl.multiple_of(i * R, R)
        carry = scan(r0, *carry)
        hidden(r0)
        return carry

    def out_copy(i, n0):
        return pltpu.make_async_copy(ost.at[i, :, pl.ds(n0, _NO)],
                                     o_hbm.at[pl.ds(i * R, R), pl.ds(n0, _NO)], sem_o)

    def cproj(r0, n0):
        a = None
        for l in range(8):
            ks = slice(l * 128, (l + 1) * 128)
            rows = pl.ds(pl.multiple_of(r0 + (l * S // 8) * 8, 8) + (l * S) % 8, R)
            t = (_dot_nt(hre[rows, :].astype(_bf16), cre_s[n0:n0 + _NO, ks])
                 + _dot_nt(him[rows, :].astype(_bf16), cim_s[n0:n0 + _NO, ks]))
            a = t if a is None else a + t
        return a

    def loop_b(i, c):
        r0 = pl.multiple_of(i * R, R)
        h = hg[pl.ds(r0, R), :]
        for n0 in range(0, _D, _NO):
            b = _dot(h, wd_s[:, n0:n0 + _NO])
            a = cproj(r0, n0)
            gate = jnp.concatenate([gs[pl.ds(r0, R), :]] * (_NO // 128), axis=1)
            xf = xs[pl.ds(r0, R), n0:n0 + _NO].astype(_f32)
            a = a + xf * _tile(dk[0, :, n0:n0 + _NO], R // 8)
            ost[i, :, n0:n0 + _NO] = gate * a + (1.0 - gate) * b
            out_copy(i, n0).start()
        return c

    z = jnp.zeros((8, 128), _f32)
    wait(w_copies()[:2])
    lax.fori_loop(0, _NBLK, loop_a, (z, z))
    wait(w_copies()[2:])
    lax.fori_loop(0, _NBLK, loop_b, 0)
    pltpu.make_async_copy(ost, ost, sem_o).wait()


@jax.jit
def pallas_gated_mix__ssm_conv_s5__glu_gated_geglu__prompt_kernel(
    A_x: jax.Array,
    A_Lambda_re: jax.Array,
    A_Lambda_im: jax.Array,
    A_B_re: jax.Array,
    A_B_im: jax.Array,
    A_C_re: jax.Array,
    A_C_im: jax.Array,
    A_log_dt: jax.Array,
    A_Dskip: jax.Array,
    B_x: jax.Array,
    B_w_gate: jax.Array,
    B_w_up: jax.Array,
    B_w_down: jax.Array,
    gate_w: jax.Array,
):
    del B_x
    vec = lambda a: a.reshape(8, 128)
    any_spec = pl.BlockSpec(memory_space=pl.ANY)
    out = pl.pallas_call(
        _kernel,
        in_specs=[any_spec] * 13,
        out_specs=any_spec,
        out_shape=jax.ShapeDtypeStruct((_L, _D), _f32),
        scratch_shapes=[
            pltpu.VMEM((_L, _D), _bf16),
            pltpu.VMEM((_P, _D), _bf16),
            pltpu.VMEM((_P, _D), _bf16),
            pltpu.VMEM((_D, _P), _bf16),
            pltpu.VMEM((_D, _P), _bf16),
            pltpu.VMEM((_D, _F), _bf16),
            pltpu.VMEM((_D, _F), _bf16),
            pltpu.VMEM((_F, _D), _bf16),
            pltpu.VMEM((5, 8, 128), _bf16),
            pltpu.VMEM((2, 8, 128), _f32),
            pltpu.VMEM((2, 8, _D), _f32),
            pltpu.VMEM((2, 8, 8, 128), _f32),
            pltpu.VMEM((_L, 128), _f32),
            pltpu.VMEM((8 * _S, 128), _f32),
            pltpu.VMEM((8 * _S, 128), _f32),
            pltpu.VMEM((8 * _S, 128), _f32),
            pltpu.VMEM((8 * _S, 128), _f32),
            pltpu.VMEM((_L, _F), _bf16),
            pltpu.VMEM((_NBLK, _R, _D), _f32),
            pltpu.SemaphoreType.DMA((_NSEM,)),
            pltpu.SemaphoreType.DMA(()),
        ],
        compiler_params=pltpu.CompilerParams(vmem_limit_bytes=120 * 2**20),
        name="fused",
    )(A_x.reshape(_L, _D), vec(A_Lambda_re), vec(A_Lambda_im), vec(A_log_dt), vec(A_Dskip), vec(gate_w),
      A_B_re, A_B_im, A_C_re, A_C_im, B_w_gate, B_w_up, B_w_down)
    return out.reshape(1, _L, _D)
```

```python
import jax
import jax.numpy as jnp
from jax import lax
from jax.experimental import pallas as pl
from jax.experimental.pallas import tpu as pltpu

_L, _D, _P, _F = 2048, 1024, 1024, 3584
_R = 256
_NBLK = _L // _R
_FC = 256
_NA = 128
_NB = 256
_PIECE = 64
_GR = _R // 8
_SA = _R + 4
_SB = _L - _R + 4
_SH = _R + _PIECE + 4
_SX0, _SX1, _SXR, _SBT, _SV, _SW, _NSEM = 0, 1, 2, 3, 19, 24, 29

_f32, _bf16, _u32 = jnp.float32, jnp.bfloat16, jnp.uint32


def _dot(a, b):
    return jnp.dot(a, b, preferred_element_type=_f32)


def _dot_nt(a, b):
    return lax.dot_general(a, b, (((1,), (1,)), ((), ())), preferred_element_type=_f32)


def _gelu(x):
    c = 0.7978845608028654
    return 0.5 * x * (1.0 + jnp.tanh(c * (x + 0.044715 * (x * x * x))))


def _align(v, m):
    return v if isinstance(v, int) else pl.multiple_of(v, m)


def _rows(v, n):
    return jnp.concatenate([v] * n, axis=0)


def _cols(v, n):
    return v if n == 1 else jnp.concatenate([v] * n, axis=1)


def _kernel(x_hbm, lre_hbm, lim_hbm, ldt_hbm, dsk_hbm, gw_hbm,
            bre_hbm, bim_hbm, cre_hbm, cim_hbm, wg_hbm, wu_hbm, wd_hbm, o_hbm,
            xs, bre_s, bim_s, cre_s, cim_s, wg_s, wu_s, wd_s, vec_s,
            par, dk, cf, gs, ar_s, ai_s, br_s, bi_s, hre, him, hg, ost, sem, sem_o):
    R = _R

    def x_copy(r0, nr, k):
        return pltpu.make_async_copy(x_hbm.at[pl.ds(r0, nr), :], xs.at[pl.ds(r0, nr), :], sem.at[k])

    def b_copy(l, k):
        src, dst = ((bre_hbm, bre_s), (bim_hbm, bim_s))[k]
        rows = pl.ds(_align(l * 128, 128), 128)
        return pltpu.make_async_copy(src.at[rows, :], dst.at[rows, :], sem.at[_SBT + 2 * l + k])

    def b_copies(l):
        return [b_copy(l, 0), b_copy(l, 1)]

    def vec_copies():
        return [pltpu.make_async_copy(v, vec_s.at[k], sem.at[_SV + k])
                for k, v in enumerate((lre_hbm, lim_hbm, ldt_hbm, dsk_hbm, gw_hbm))]

    def w_copies():
        return [pltpu.make_async_copy(src, dst, sem.at[_SW + k]) for k, (src, dst) in enumerate(
            ((wg_hbm, wg_s), (wu_hbm, wu_s), (cre_hbm, cre_s), (cim_hbm, cim_s), (wd_hbm, wd_s)))]

    def out_copy(i, n0):
        return pltpu.make_async_copy(ost.at[i, :, pl.ds(n0, _NB)],
                                     o_hbm.at[pl.ds(i * R, R), pl.ds(n0, _NB)], sem_o)

    def start(cs):
        for c in cs:
            c.start()

    def wait(cs):
        for c in cs:
            c.wait()

    start([x_copy(0, R, _SX0)] + b_copies(0) + vec_copies() + [x_copy(R, R, _SX1)])
    for l in range(1, 8):
        start(b_copies(l))
    start([x_copy(2 * R, _L - 2 * R, _SXR)] + w_copies())

    def params():
        lre = vec_s[0].astype(_f32)
        lim = vec_s[1].astype(_f32)
        dt = jnp.exp(vec_s[2].astype(_f32)).astype(_bf16).astype(_f32)
        mag = jnp.exp(dt * lre)
        ang = dt * lim
        ar = mag * jnp.cos(ang)
        ai = mag * jnp.sin(ang)
        nr = ar - 1.0
        den = 2.0 / (lre * lre + lim * lim)
        cr = (nr * lre + ai * lim) * den
        ci = (ai * lre - nr * lim) * den
        par[0] = ar
        par[1] = ai
        dsk = vec_s[3].astype(_f32)
        gw = vec_s[4].astype(_f32)
        for l in range(8):
            sl = slice(l * 128, (l + 1) * 128)
            dk[0, :, sl] = jnp.broadcast_to(dsk[l:l + 1, :], (8, 128))
            dk[1, :, sl] = jnp.broadcast_to(gw[l:l + 1, :], (8, 128))
            cf[0, l] = jnp.broadcast_to(cr[l:l + 1, :], (8, 128))
            cf[1, l] = jnp.broadcast_to(ci[l:l + 1, :], (8, 128))

    def gate_rows(r0, nr):
        xf = xs[pl.ds(r0, nr), :].astype(_f32)
        s = jnp.sum(xf * _rows(dk[1], nr // 8), axis=-1, keepdims=True)
        g = jnp.broadcast_to(jax.nn.sigmoid(s), (nr, 128))
        gs[pl.ds(r0, nr), :] = g
        return g

    def bu_dot(r0, l, w_s):
        return _dot_nt(xs[pl.ds(r0, R), :], w_s[pl.ds(_align(l * 128, 128), 128), :])

    def bu_fin(r0, l0, k, b_r, b_i):
        l = l0 + k
        c_r = cf[0, l]
        c_i = cf[1, l]
        g = gate_rows(_align(r0 + l * _GR, _GR), _GR)
        w = lax.bitcast_convert_type(g, _u32)
        m = w[0:8]
        for j in range(1, _GR // 8):
            m = m | w[8 * j:8 * j + 8]
        c_r = _rows(jnp.where((m | 1) != 0, c_r, 0.0), R // 8)
        c_i = _rows(c_i, R // 8)
        if isinstance(r0, int) and r0 == 0:
            re_s, im_s, s, q0 = ar_s, ai_s, _SA, 0
        else:
            re_s, im_s, s, q0 = br_s, bi_s, _SB, r0 - R
        base = _align(l0 * s + q0 + (k * s // 8) * 8, 8) + (k * s) % 8
        re_s[pl.ds(base, R), :] = c_r * b_r - c_i * b_i
        im_s[pl.ds(base, R), :] = -(c_r * b_i + c_i * b_r)

    def bu(r0, l0, k):
        bu_fin(r0, l0, k, bu_dot(r0, l0 + k, bre_s), bu_dot(r0, l0 + k, bim_s))

    def scan(re_s, im_s, s, q0, w0, n, hr, hi):
        ar, ai = par[0], par[1]
        for t in range(n):
            b_r = re_s[pl.ds(q0 + t, 8, stride=s), :]
            b_i = im_s[pl.ds(q0 + t, 8, stride=s), :]
            hr, hi = ar * hr + ai * hi + b_r, ar * hi - ai * hr + b_i
            hre[pl.ds(w0 + t, 8, stride=_SH), :] = hr
            him[pl.ds(w0 + t, 8, stride=_SH), :] = hi
        return hr, hi

    wait([x_copy(0, R, _SX0), b_copy(0, 0)])
    first_r = bu_dot(0, 0, bre_s)
    wait([b_copy(0, 1)])
    first_i = bu_dot(0, 0, bim_s)
    wait([x_copy(R, R, _SX1)] + vec_copies())
    params()
    bu_fin(0, 0, 0, first_r, first_i)
    bu(R, 0, 0)
    wait(b_copies(1))
    bu(0, 0, 1)
    bu(R, 0, 1)

    def first_blocks(j, c):
        l0 = 2 * j
        wait(b_copies(l0) + b_copies(l0 + 1))
        for k in range(2):
            bu(0, l0, k)
            bu(R, l0, k)
        return c

    lax.fori_loop(1, 4, first_blocks, 0)
    wait([x_copy(2 * R, _L - 2 * R, _SXR)])

    def other_blocks(i, carry):
        r0 = pl.multiple_of(i * R, R)
        for l in range(8):
            bu(r0, 0, l)
        j = i - 2
        npc = R // _PIECE
        q0 = pl.multiple_of(jnp.minimum(j, npc - 1) * _PIECE, _PIECE)
        w0 = pl.multiple_of(jnp.minimum(j, npc) * _PIECE, _PIECE)
        hr, hi = scan(ar_s, ai_s, _SA, q0, w0, _PIECE, *carry)
        return jnp.where(j < npc, hr, carry[0]), jnp.where(j < npc, hi, carry[1])

    z = jnp.zeros((8, 128), _f32)
    state = lax.fori_loop(2, _NBLK, other_blocks, (z, z))

    def ssm_out(n0):
        a = None
        for l in range(8):
            ks = slice(l * 128, (l + 1) * 128)
            rows = pl.ds(l * _SH, R)
            t = (_dot_nt(hre[rows, :].astype(_bf16), cre_s[n0:n0 + _NA, ks])
                 + _dot_nt(him[rows, :].astype(_bf16), cim_s[n0:n0 + _NA, ks]))
            a = t if a is None else a + t
        return a

    def block(i, carry):
        r0 = pl.multiple_of(i * R, R)
        for n0 in range(0, _D, _NA):
            xf = xs[pl.ds(r0, R), n0:n0 + _NA].astype(_f32)
            a = ssm_out(n0) + xf * _rows(dk[0, :, n0:n0 + _NA], R // 8)
            ost[i, :, n0:n0 + _NA] = _cols(gs[pl.ds(r0, R), :], _NA // 128) * a
        q0 = pl.multiple_of(jnp.minimum(i, _NBLK - 2) * R, R)
        carry = scan(br_s, bi_s, _SB, q0, 0, R, *carry)
        x = xs[pl.ds(r0, R), :]
        for f0 in range(0, _F, _FC):
            g = _dot(x, wg_s[:, f0:f0 + _FC])
            u = _dot(x, wu_s[:, f0:f0 + _FC])
            hg[:, f0:f0 + _FC] = (_gelu(g) * u).astype(_bf16)
        for n0 in range(0, _D, _NB):
            b = _dot(hg[...], wd_s[:, n0:n0 + _NB])
            gate = _cols(gs[pl.ds(r0, R), :], _NB // 128)
            ost[i, :, n0:n0 + _NB] = ost[i, :, n0:n0 + _NB] + (1.0 - gate) * b
            out_copy(i, n0).start()
        return carry

    wait(w_copies())
    lax.fori_loop(0, _NBLK, block, state)
    pltpu.make_async_copy(ost, ost, sem_o).wait()


@jax.jit
def pallas_gated_mix__ssm_conv_s5__glu_gated_geglu__prompt_kernel(
    A_x: jax.Array,
    A_Lambda_re: jax.Array,
    A_Lambda_im: jax.Array,
    A_B_re: jax.Array,
    A_B_im: jax.Array,
    A_C_re: jax.Array,
    A_C_im: jax.Array,
    A_log_dt: jax.Array,
    A_Dskip: jax.Array,
    B_x: jax.Array,
    B_w_gate: jax.Array,
    B_w_up: jax.Array,
    B_w_down: jax.Array,
    gate_w: jax.Array,
):
    del B_x
    vec = lambda a: a.reshape(8, 128)
    any_spec = pl.BlockSpec(memory_space=pl.ANY)
    out = pl.pallas_call(
        _kernel,
        in_specs=[any_spec] * 13,
        out_specs=any_spec,
        out_shape=jax.ShapeDtypeStruct((_L, _D), _f32),
        scratch_shapes=[
            pltpu.VMEM((_L, _D), _bf16),
            pltpu.VMEM((_P, _D), _bf16),
            pltpu.VMEM((_P, _D), _bf16),
            pltpu.VMEM((_D, _P), _bf16),
            pltpu.VMEM((_D, _P), _bf16),
            pltpu.VMEM((_D, _F), _bf16),
            pltpu.VMEM((_D, _F), _bf16),
            pltpu.VMEM((_F, _D), _bf16),
            pltpu.VMEM((5, 8, 128), _bf16),
            pltpu.VMEM((2, 8, 128), _f32),
            pltpu.VMEM((2, 8, _D), _f32),
            pltpu.VMEM((2, 8, 8, 128), _f32),
            pltpu.VMEM((_L, 128), _f32),
            pltpu.VMEM((8 * _SA, 128), _f32),
            pltpu.VMEM((8 * _SA, 128), _f32),
            pltpu.VMEM((8 * _SB, 128), _f32),
            pltpu.VMEM((8 * _SB, 128), _f32),
            pltpu.VMEM((8 * _SH, 128), _f32),
            pltpu.VMEM((8 * _SH, 128), _f32),
            pltpu.VMEM((_R, _F), _bf16),
            pltpu.VMEM((_NBLK, _R, _D), _f32),
            pltpu.SemaphoreType.DMA((_NSEM,)),
            pltpu.SemaphoreType.DMA(()),
        ],
        compiler_params=pltpu.CompilerParams(vmem_limit_bytes=120 * 2**20),
        name="fused",
    )(A_x.reshape(_L, _D), vec(A_Lambda_re), vec(A_Lambda_im), vec(A_log_dt), vec(A_Dskip), vec(gate_w),
      A_B_re, A_B_im, A_C_re, A_C_im, B_w_gate, B_w_up, B_w_down)
    return out.reshape(1, _L, _D)
```

```python
import jax
import jax.numpy as jnp
from jax import lax
from jax.experimental import pallas as pl
from jax.experimental.pallas import tpu as pltpu

_L, _D, _P, _F = 2048, 1024, 1024, 3584
_R = 256
_NBLK = _L // _R
_FC = 128
_NC = 128
_PIECE = 64
_GR = _R // 8
_SA = _R + 4
_SB = _L - _R + 4
_SH = _R + 4
_SX0, _SX1, _SXR, _SBT, _SV, _SW, _NSEM = 0, 1, 2, 3, 19, 24, 29

_f32, _bf16, _u32 = jnp.float32, jnp.bfloat16, jnp.uint32


def _dot(a, b):
    return jnp.dot(a, b, preferred_element_type=_f32)


def _dot_nt(a, b):
    return lax.dot_general(a, b, (((1,), (1,)), ((), ())), preferred_element_type=_f32)


def _gelu(x):
    c = 0.7978845608028654
    return 0.5 * x * (1.0 + jnp.tanh(c * (x + 0.044715 * (x * x * x))))


def _align(v, m):
    return v if isinstance(v, int) else pl.multiple_of(v, m)


def _rows(v, n):
    return jnp.concatenate([v] * n, axis=0)


def _kernel(x_hbm, lre_hbm, lim_hbm, ldt_hbm, dsk_hbm, gw_hbm,
            bre_hbm, bim_hbm, cre_hbm, cim_hbm, wg_hbm, wu_hbm, wd_hbm, o_hbm,
            xs, bre_s, bim_s, cre_s, cim_s, wg_s, wu_s, wd_s, vec_s,
            par, dk, cf, gs, ar_s, ai_s, br_s, bi_s, hre, him, hg, ost, sem, sem_o):
    R = _R

    def x_copy(r0, nr, k):
        return pltpu.make_async_copy(x_hbm.at[pl.ds(r0, nr), :], xs.at[pl.ds(r0, nr), :], sem.at[k])

    def b_copy(l, k):
        src, dst = ((bre_hbm, bre_s), (bim_hbm, bim_s))[k]
        rows = pl.ds(_align(l * 128, 128), 128)
        return pltpu.make_async_copy(src.at[rows, :], dst.at[rows, :], sem.at[_SBT + 2 * l + k])

    def b_copies(l):
        return [b_copy(l, 0), b_copy(l, 1)]

    def vec_copies():
        return [pltpu.make_async_copy(v, vec_s.at[k], sem.at[_SV + k])
                for k, v in enumerate((lre_hbm, lim_hbm, ldt_hbm, dsk_hbm, gw_hbm))]

    def w_copies():
        return [pltpu.make_async_copy(src, dst, sem.at[_SW + k]) for k, (src, dst) in enumerate(
            ((wg_hbm, wg_s), (wu_hbm, wu_s), (cre_hbm, cre_s), (cim_hbm, cim_s), (wd_hbm, wd_s)))]

    def out_copy(i, n0):
        return pltpu.make_async_copy(ost.at[i, :, pl.ds(n0, _NC)],
                                     o_hbm.at[pl.ds(i * R, R), pl.ds(n0, _NC)], sem_o)

    def start(cs):
        for c in cs:
            c.start()

    def wait(cs):
        for c in cs:
            c.wait()

    start([x_copy(0, R, _SX0)] + b_copies(0) + vec_copies() + [x_copy(R, R, _SX1)])
    for l in range(1, 8):
        start(b_copies(l))
    start([x_copy(2 * R, _L - 2 * R, _SXR)] + w_copies())

    def params():
        lre = vec_s[0].astype(_f32)
        lim = vec_s[1].astype(_f32)
        dt = jnp.exp(vec_s[2].astype(_f32)).astype(_bf16).astype(_f32)
        mag = jnp.exp(dt * lre)
        ang = dt * lim
        ar = mag * jnp.cos(ang)
        ai = mag * jnp.sin(ang)
        nr = ar - 1.0
        den = 2.0 / (lre * lre + lim * lim)
        cr = (nr * lre + ai * lim) * den
        ci = (ai * lre - nr * lim) * den
        par[0] = ar
        par[1] = ai
        dsk = vec_s[3].astype(_f32)
        gw = vec_s[4].astype(_f32)
        for l in range(8):
            sl = slice(l * 128, (l + 1) * 128)
            dk[0, :, sl] = jnp.broadcast_to(dsk[l:l + 1, :], (8, 128))
            dk[1, :, sl] = jnp.broadcast_to(gw[l:l + 1, :], (8, 128))
            cf[0, l] = jnp.broadcast_to(cr[l:l + 1, :], (8, 128))
            cf[1, l] = jnp.broadcast_to(ci[l:l + 1, :], (8, 128))

    def gate_rows(r0, nr):
        xf = xs[pl.ds(r0, nr), :].astype(_f32)
        s = jnp.sum(xf * _rows(dk[1], nr // 8), axis=-1, keepdims=True)
        g = jnp.broadcast_to(jax.nn.sigmoid(s), (nr, 128))
        gs[pl.ds(r0, nr), :] = g
        return g

    def bu_dot(r0, l, w_s):
        return _dot_nt(xs[pl.ds(r0, R), :], w_s[pl.ds(_align(l * 128, 128), 128), :])

    def bu_fin(r0, l0, k, b_r, b_i):
        l = l0 + k
        c_r = cf[0, l]
        c_i = cf[1, l]
        g = gate_rows(_align(r0 + l * _GR, _GR), _GR)
        w = lax.bitcast_convert_type(g, _u32)
        m = w[0:8]
        for j in range(1, _GR // 8):
            m = m | w[8 * j:8 * j + 8]
        c_r = _rows(jnp.where((m | 1) != 0, c_r, 0.0), R // 8)
        c_i = _rows(c_i, R // 8)
        if isinstance(r0, int) and r0 == 0:
            re_s, im_s, s, q0 = ar_s, ai_s, _SA, 0
        else:
            re_s, im_s, s, q0 = br_s, bi_s, _SB, r0 - R
        base = _align(l0 * s + q0 + (k * s // 8) * 8, 8) + (k * s) % 8
        re_s[pl.ds(base, R), :] = c_r * b_r - c_i * b_i
        im_s[pl.ds(base, R), :] = -(c_r * b_i + c_i * b_r)

    def bu(r0, l0, k):
        bu_fin(r0, l0, k, bu_dot(r0, l0 + k, bre_s), bu_dot(r0, l0 + k, bim_s))

    def scan(re_s, im_s, s, q0, w0, n, hr, hi):
        ar, ai = par[0], par[1]
        for t in range(n):
            b_r = re_s[pl.ds(q0 + t, 8, stride=s), :]
            b_i = im_s[pl.ds(q0 + t, 8, stride=s), :]
            hr, hi = ar * hr + ai * hi + b_r, ar * hi - ai * hr + b_i
            hre[pl.ds(w0 + t, 8, stride=_SH), :] = hr
            him[pl.ds(w0 + t, 8, stride=_SH), :] = hi
        return hr, hi

    wait([x_copy(0, R, _SX0), b_copy(0, 0)])
    first_r = bu_dot(0, 0, bre_s)
    wait([b_copy(0, 1)])
    first_i = bu_dot(0, 0, bim_s)
    wait([x_copy(R, R, _SX1)] + vec_copies())
    params()
    bu_fin(0, 0, 0, first_r, first_i)
    bu(R, 0, 0)
    wait(b_copies(1))
    bu(0, 0, 1)
    bu(R, 0, 1)

    def first_blocks(j, c):
        l0 = 2 * j
        wait(b_copies(l0) + b_copies(l0 + 1))
        for k in range(2):
            bu(0, l0, k)
            bu(R, l0, k)
        return c

    lax.fori_loop(1, 4, first_blocks, 0)
    wait([x_copy(2 * R, _L - 2 * R, _SXR)])

    def other_blocks(j, carry):
        for k in range(12):
            n = 12 * j + k
            r0 = pl.multiple_of((2 + n // 8) * R, R)
            l0 = lax.rem(n - (k % 2), 8)
            bu(r0, l0, k % 2)
        q0 = pl.multiple_of(j * _PIECE, _PIECE)
        return scan(ar_s, ai_s, _SA, q0, q0, _PIECE, *carry)

    z = jnp.zeros((8, 128), _f32)
    state = lax.fori_loop(0, 4, other_blocks, (z, z))

    def block(i, carry):
        r0 = pl.multiple_of(i * R, R)
        hs = [(hre[pl.ds(l * _SH, R), :].astype(_bf16), him[pl.ds(l * _SH, R), :].astype(_bf16))
              for l in range(8)]
        x = xs[pl.ds(r0, R), :]
        for f0 in range(0, _F, _FC):
            g = _dot(x, wg_s[:, f0:f0 + _FC])
            u = _dot(x, wu_s[:, f0:f0 + _FC])
            hg[:, f0:f0 + _FC] = (_gelu(g) * u).astype(_bf16)
        for n0 in range(0, _D, _NC):
            a = xs[pl.ds(r0, R), n0:n0 + _NC].astype(_f32) * _rows(dk[0, :, n0:n0 + _NC], R // 8)
            y = None
            for l in range(8):
                ks = slice(l * 128, (l + 1) * 128)
                t = (_dot_nt(hs[l][0], cre_s[n0:n0 + _NC, ks]) + _dot_nt(hs[l][1], cim_s[n0:n0 + _NC, ks]))
                y = t if y is None else y + t
            ost[i, :, n0:n0 + _NC] = gs[pl.ds(r0, R), :] * (y + a)
        q0 = pl.multiple_of(jnp.minimum(i, _NBLK - 2) * R, R)
        carry = scan(br_s, bi_s, _SB, q0, 0, R, *carry)
        for n0 in range(0, _D, _NC):
            b = _dot(hg[...], wd_s[:, n0:n0 + _NC])
            ost[i, :, n0:n0 + _NC] = ost[i, :, n0:n0 + _NC] + (1.0 - gs[pl.ds(r0, R), :]) * b
            out_copy(i, n0).start()
        return carry

    wait(w_copies())
    lax.fori_loop(0, _NBLK, block, state)
    pltpu.make_async_copy(ost, ost, sem_o).wait()


@jax.jit
def pallas_gated_mix__ssm_conv_s5__glu_gated_geglu__prompt_kernel(
    A_x: jax.Array,
    A_Lambda_re: jax.Array,
    A_Lambda_im: jax.Array,
    A_B_re: jax.Array,
    A_B_im: jax.Array,
    A_C_re: jax.Array,
    A_C_im: jax.Array,
    A_log_dt: jax.Array,
    A_Dskip: jax.Array,
    B_x: jax.Array,
    B_w_gate: jax.Array,
    B_w_up: jax.Array,
    B_w_down: jax.Array,
    gate_w: jax.Array,
):
    del B_x
    vec = lambda a: a.reshape(8, 128)
    any_spec = pl.BlockSpec(memory_space=pl.ANY)
    out = pl.pallas_call(
        _kernel,
        in_specs=[any_spec] * 13,
        out_specs=any_spec,
        out_shape=jax.ShapeDtypeStruct((_L, _D), _f32),
        scratch_shapes=[
            pltpu.VMEM((_L, _D), _bf16),
            pltpu.VMEM((_P, _D), _bf16),
            pltpu.VMEM((_P, _D), _bf16),
            pltpu.VMEM((_D, _P), _bf16),
            pltpu.VMEM((_D, _P), _bf16),
            pltpu.VMEM((_D, _F), _bf16),
            pltpu.VMEM((_D, _F), _bf16),
            pltpu.VMEM((_F, _D), _bf16),
            pltpu.VMEM((5, 8, 128), _bf16),
            pltpu.VMEM((2, 8, 128), _f32),
            pltpu.VMEM((2, 8, _D), _f32),
            pltpu.VMEM((2, 8, 8, 128), _f32),
            pltpu.VMEM((_L, 128), _f32),
            pltpu.VMEM((8 * _SA, 128), _f32),
            pltpu.VMEM((8 * _SA, 128), _f32),
            pltpu.VMEM((8 * _SB, 128), _f32),
            pltpu.VMEM((8 * _SB, 128), _f32),
            pltpu.VMEM((8 * _SH, 128), _f32),
            pltpu.VMEM((8 * _SH, 128), _f32),
            pltpu.VMEM((_R, _F), _bf16),
            pltpu.VMEM((_NBLK, _R, _D), _f32),
            pltpu.SemaphoreType.DMA((_NSEM,)),
            pltpu.SemaphoreType.DMA(()),
        ],
        compiler_params=pltpu.CompilerParams(vmem_limit_bytes=120 * 2**20),
        name="fused",
    )(A_x.reshape(_L, _D), vec(A_Lambda_re), vec(A_Lambda_im), vec(A_log_dt), vec(A_Dskip), vec(gate_w),
      A_B_re, A_B_im, A_C_re, A_C_im, B_w_gate, B_w_up, B_w_down)
    return out.reshape(1, _L, _D)
```
